```python
import os as _os
_os.environ.setdefault("JAX_PLATFORMS", "cpu")
import jax
import jax.numpy as jnp

def _softmax(x, axis=-1):
    return jax.nn.softmax(x, axis=axis)
def _gelu(x):
    return jax.nn.gelu(x, approximate=True)
def _silu(x):
    return jax.nn.silu(x)
def _sigmoid(x):
    return jax.nn.sigmoid(x)
def _layernorm(x, axis=-1, eps=1e-5):
    m = jnp.mean(x, axis=axis, keepdims=True)
    v = jnp.var(x, axis=axis, keepdims=True)
    return (x - m) / jnp.sqrt(v + eps)
def _scatter_add(tgt, idx, src, axis=0):
    return tgt.at[idx].add(src)
def _segment_sum(src, seg, n):
    return jax.ops.segment_sum(src, seg, n)
class _Rng:
    def __init__(self, key):
        self._k = key
    def _next(self):
        self._k, sub = jax.random.split(self._k)
        return sub
    def normal(self, shape):
        return jax.random.normal(self._next(), shape, dtype=jnp.bfloat16)
    def randint(self, lo, hi, shape):
        return jax.random.randint(self._next(), shape, lo, hi, dtype=jnp.int32)
    def uniform(self, shape, lo=0.0, hi=1.0):
        return jax.random.uniform(self._next(), shape, jnp.bfloat16, lo, hi)
    def permutation(self, n):
        return jax.random.permutation(self._next(), n)


kernel_name = 'interleave_layers__grouped_kv_mqa__sliding_block__prompt'

def setup_inputs():
    _rng = _Rng(jax.random.key(int.from_bytes(__import__("os").urandom(4), "little")))
    _w = (lambda a: (lambda t: t.astype(jnp.bfloat16) if jnp.issubdtype(t.dtype, jnp.floating) else t)(jnp.asarray(a)))
    def _A_setup():
        B, S, D, H = 1, 2048, 448, 16
        Dh = D // H
        return {
            "x": _w((lambda *s: _rng.normal(s) * 0.05)(B, S, D)),
            "wq": _w((lambda *s: _rng.normal(s) * 0.05)(D, H * Dh)),
            "wk": _w((lambda *s: _rng.normal(s) * 0.05)(D, Dh)),
            "wv": _w((lambda *s: _rng.normal(s) * 0.05)(D, Dh)),
            "wo": _w((lambda *s: _rng.normal(s) * 0.05)(H * Dh, D)),
        }
    _A_in = _A_setup()

    def _B_setup():
        B, S, D = 1, 2048, 448
        return {
            "x": _w((lambda *s: _rng.normal(s) * 0.05)(B, S, D)),
            "wqkv": _w((lambda *s: _rng.normal(s) * 0.05)(D, 3 * D)),
            "wo": _w((lambda *s: _rng.normal(s) * 0.05)(D, D)),
        }
    _B_in = _B_setup()

    return {
        "A_x": _A_in["x"],
        "A_wq": _A_in["wq"],
        "A_wk": _A_in["wk"],
        "A_wv": _A_in["wv"],
        "A_wo": _A_in["wo"],
        "B_x": _B_in["x"],
        "B_wqkv": _B_in["wqkv"],
        "B_wo": _B_in["wo"],
    }

def reference(A_x, A_wq, A_wk, A_wv, A_wo, B_x, B_wqkv, B_wo):
    def _A_ref(x, wq, wk, wv, wo):
        B, S, D = x.shape
        H = 16
        Dh = D // H
        q = (lambda x, *d: x.transpose(*d))((x @ wq).reshape(B, S, H, Dh), 0, 2, 1, 3)
        k = x @ wk
        v = x @ wv
        scores = jnp.einsum("bhqd,bkd->bhqk", q, k) * (Dh ** -0.5)
        p = _softmax(scores, axis=-1)
        o = jnp.einsum("bhqk,bkd->bhqd", p, v)
        return (lambda x, *d: x.transpose(*d))(o, 0, 2, 1, 3).reshape(B, S, H * Dh) @ wo

    def _B_ref(x, wqkv, wo):
        B, S, D = x.shape
        H = 16; Dh = D // H; W = 256
        qkv = (lambda x, *d: x.transpose(*d))((x @ wqkv).reshape(B, S, 3, H, Dh), 2, 0, 3, 1, 4)
        q, k, v = qkv[0], qkv[1], qkv[2]
        scores = jnp.einsum("bhqd,bhkd->bhqk", q, k) * (Dh ** -0.5)
        idx = jnp.arange(S)
        mask = (idx[:, None] - idx[None, :] >= 0) & (idx[:, None] - idx[None, :] < W)
        scores = jnp.where(mask[None, None], scores, -1e9)
        p = _softmax(scores, axis=-1)
        o = jnp.einsum("bhqk,bhkd->bhqd", p, v)
        return (lambda x, *d: x.transpose(*d))(o, 0, 2, 1, 3).reshape(B, S, D) @ wo

    x = A_x
    x = x + _A_ref(_layernorm(x, axis=-1), A_wq, A_wk, A_wv, A_wo)
    x = x + _B_ref(_layernorm(x, axis=-1), B_wqkv, B_wo)
    x = x + _A_ref(_layernorm(x, axis=-1), A_wq, A_wk, A_wv, A_wo)
    x = x + _B_ref(_layernorm(x, axis=-1), B_wqkv, B_wo)
    return x
```

```python
import functools
import math

import jax
import jax.numpy as jnp
from jax import lax
import jax.experimental.pallas as pl
import jax.experimental.pallas.tpu as pltpu

S = 2048
D = 448
H = 16
DH = 28
HP = 32
G = 4
GR = G * DH
TB = 512
NB = S // TB
WIN = 256
QSCALE = (DH ** -0.5) * math.log2(math.e)
EPS = 1e-5
F32 = jnp.float32
BF16 = jnp.bfloat16


def _dot(a, b):
    return jnp.dot(a, b, preferred_element_type=F32)


def _layernorm_t(x):
    mean = jnp.sum(x, axis=0, keepdims=True) * (1.0 / D)
    xc = x - mean
    var = jnp.sum(xc * xc, axis=0, keepdims=True) * (1.0 / D)
    return xc * lax.rsqrt(var + EPS)


def make_kernel(a_unroll=4, a_ch=128):
    def kernel(xT_ref, wq_ref, wkT_ref, wvT_ref, woA_ref, wqkv_ref, woB_ref, o_ref,
               xs, xn, wA, woAT, wB, woBT, qs, kz, vt, os_, ss):
        def put_wT(dst, row0, w):
            dst[row0:row0 + w.shape[1], :] = w.astype(F32).T.astype(BF16)

        put_wT(wA, 0, wq_ref[...])
        z4 = jnp.zeros((HP - DH, D), F32)
        wA[D:D + 2 * HP, :] = jnp.concatenate(
            [wkT_ref[...].astype(F32), z4, wvT_ref[...].astype(F32), z4], axis=0).astype(BF16)
        for c in range(3):
            put_wT(wB, c * D, wqkv_ref[:, c * D:(c + 1) * D])

        def pad_woT(dst, w_ref):
            w = w_ref[...].astype(F32)
            parts = []
            for h in range(H):
                parts += [w[h * DH:(h + 1) * DH], z4]
            dst[...] = jnp.concatenate(parts, axis=0).T.astype(BF16)

        pad_woT(woAT, woA_ref)
        pad_woT(woBT, woB_ref)

        for b in range(NB):
            x = xT_ref[:, b * TB:(b + 1) * TB].astype(F32)
            xs[b] = x
            xn[b] = _layernorm_t(x).astype(BF16)

        row32 = lax.broadcasted_iota(jnp.int32, (HP, TB), 0)

        def proj_a(b):
            r = _dot(wA[...], xn[b])
            qs[b] = (r[:D] * QSCALE).astype(BF16)
            k = r[D:D + HP]
            v = jnp.where(row32 == DH, 1.0, r[D + HP:])
            vt[0:HP, b * TB:(b + 1) * TB] = v.astype(BF16)
            kp = jnp.concatenate([k, jnp.zeros((128 - HP, TB), F32)], axis=0)
            for j in range(G):
                kj = kp if j == 0 else pltpu.roll(kp, DH * j, 0)
                kz[j, b * TB:(b + 1) * TB, :] = kj.T.astype(BF16)

        def proj_b(b):
            xb = xn[b]
            q = _dot(wB[0:D], xb)
            qs[b] = (q * QSCALE).astype(BF16)
            k = _dot(wB[D:2 * D], xb)
            for g in range(G):
                kg = jnp.concatenate([k[g * GR:(g + 1) * GR], jnp.zeros((128 - GR, TB), F32)], axis=0)
                kz[g, b * TB:(b + 1) * TB, :] = kg.T.astype(BF16)
            v = _dot(wB[2 * D:3 * D], xb)
            tail = jnp.where(lax.broadcasted_iota(jnp.int32, (HP - DH, TB), 0) == 0, 1.0, 0.0).astype(F32)
            parts = []
            for h in range(H):
                parts += [v[h * DH:(h + 1) * DH], tail]
            vt[:, b * TB:(b + 1) * TB] = jnp.concatenate(parts, axis=0).astype(BF16)

        def out_proj(b, woT, last):
            x = xs[b] + _dot(woT[...], os_[b])
            if last:
                o_ref[:, b * TB:(b + 1) * TB] = x.astype(o_ref.dtype)
            else:
                xs[b] = x
                xn[b] = _layernorm_t(x).astype(BF16)

        def attn_a():
            nch = S // a_ch

            def load_q(i):
                h = i // NB
                b = i % NB
                q = qs[b, pl.ds(pl.multiple_of((h // G) * GR, 16), GR), :]
                return q, h % G

            def qk(c, q, j):
                return _dot(kz[j, c * a_ch:(c + 1) * a_ch, 0:GR], q)

            def colmax8(s):
                return jnp.max(s.reshape(a_ch // 8, 8, TB), axis=0)

            q, j = load_q(0)
            m = None
            for c in range(nch):
                s = qk(c, q, j)
                ss[c * a_ch:(c + 1) * a_ch, :] = s
                mm = colmax8(s)
                m = mm if m is None else jnp.maximum(m, mm)
            m0 = jnp.max(m, axis=0, keepdims=True)
            nstep = H * NB

            def finish(i, acc):
                o = acc * (1.0 / acc[DH:DH + 1, :])
                os_[i % NB, pl.ds(pl.multiple_of((i // NB) * HP, HP), HP), :] = o.astype(BF16)

            def body(i, m_cur):
                q, j = load_q(i + 1)
                m = None
                acc = None
                for c in range(nch):
                    sn = qk(c, q, j)
                    p = jnp.exp2(ss[c * a_ch:(c + 1) * a_ch, :] - m_cur).astype(BF16)
                    ss[c * a_ch:(c + 1) * a_ch, :] = sn
                    mm = colmax8(sn)
                    m = mm if m is None else jnp.maximum(m, mm)
                    o = _dot(vt[0:HP, c * a_ch:(c + 1) * a_ch], p)
                    acc = o if acc is None else acc + o
                finish(i, acc)
                return jnp.max(m, axis=0, keepdims=True)

            m_last = lax.fori_loop(0, nstep - 1, body, m0, unroll=a_unroll)
            acc = None
            for c in range(nch):
                p = jnp.exp2(ss[c * a_ch:(c + 1) * a_ch, :] - m_last).astype(BF16)
                o = _dot(vt[0:HP, c * a_ch:(c + 1) * a_ch], p)
                acc = o if acc is None else acc + o
            finish(nstep - 1, acc)

        def attn_b():
            nt = S // 128
            rr = lax.broadcasted_iota(jnp.int32, (128, G * 128), 0)
            cc = lax.broadcasted_iota(jnp.int32, (128, G * 128), 1) % 128
            upper = rr > cc
            qrow = lax.broadcasted_iota(jnp.int32, (GR, 128), 0)

            def body(g, _):
                g0 = pl.multiple_of(g * GR, 16)

                def qk(t):
                    qt = qs[t // 4, pl.ds(g0, GR), (t % 4) * 128:(t % 4 + 1) * 128].astype(F32)
                    w = jnp.concatenate(
                        [jnp.where((qrow >= DH * j) & (qrow < DH * (j + 1)), qt, 0.0).astype(BF16)
                         for j in range(G)], axis=1)
                    k0 = max(t - 2, 0) * 128
                    return _dot(kz[g, k0:(t + 1) * 128, 0:GR], w)

                def pv(t, s):
                    if t == 0:
                        mrg = jnp.where(upper, -jnp.inf, s)
                        mid = None
                    elif t == 1:
                        mrg = jnp.where(upper, -jnp.inf, s[128:256])
                        mid = s[0:128]
                    else:
                        mrg = jnp.where(upper, s[0:128], s[256:384])
                        mid = s[128:256]
                    m = jnp.max(mrg, axis=0, keepdims=True)
                    if mid is not None:
                        m = jnp.maximum(m, jnp.max(mid, axis=0, keepdims=True))
                    pm = jnp.exp2(mrg - m)
                    parts = []
                    if t >= 2:
                        parts.append(jnp.where(upper, pm, 0.0).astype(BF16))
                    if mid is not None:
                        parts.append(jnp.exp2(mid - m).astype(BF16))
                    parts.append(jnp.where(upper, 0.0, pm).astype(BF16) if t >= 2 else pm.astype(BF16))
                    p = jnp.concatenate(parts, axis=0) if len(parts) > 1 else parts[0]
                    k0 = max(t - 2, 0) * 128
                    for j in range(G):
                        r0 = pl.multiple_of((g * G + j) * HP, HP)
                        o = _dot(vt[pl.ds(r0, HP), k0:(t + 1) * 128], p[:, j * 128:(j + 1) * 128])
                        o = o * (1.0 / o[DH:DH + 1, :])
                        os_[t // 4, pl.ds(r0, HP), (t % 4) * 128:(t % 4 + 1) * 128] = o.astype(BF16)

                s_cur = qk(0)
                for t in range(nt):
                    s_next = qk(t + 1) if t + 1 < nt else None
                    pv(t, s_cur)
                    s_cur = s_next
                return None

            lax.fori_loop(0, G, body, None)

        def layer_pair(it, _):
            for b in range(NB):
                proj_a(b)
            attn_a()
            for b in range(NB):
                out_proj(b, woAT, False)
            for b in range(NB):
                proj_b(b)
            attn_b()
            for b in range(NB):
                out_proj(b, woBT, False)
            return None

        lax.fori_loop(0, 2, layer_pair, None)
        for b in range(NB):
            o_ref[:, b * TB:(b + 1) * TB] = xs[b].astype(o_ref.dtype)

    return kernel


def build(**kw):
    def fn(A_x, A_wq, A_wk, A_wv, A_wo, B_x, B_wqkv, B_wo):
        xT = jnp.transpose(A_x[0])
        out = pl.pallas_call(
            make_kernel(**kw),
            out_shape=jax.ShapeDtypeStruct((D, S), A_x.dtype),
            scratch_shapes=[
                pltpu.VMEM((NB, D, TB), F32),
                pltpu.VMEM((NB, D, TB), BF16),
                pltpu.VMEM((D + 2 * HP, D), BF16),
                pltpu.VMEM((D, H * HP), BF16),
                pltpu.VMEM((3 * D, D), BF16),
                pltpu.VMEM((D, H * HP), BF16),
                pltpu.VMEM((NB, D, TB), BF16),
                pltpu.VMEM((G, S, 128), BF16),
                pltpu.VMEM((H * HP, S), BF16),
                pltpu.VMEM((NB, H * HP, TB), BF16),
                pltpu.VMEM((S, TB), F32),
            ],
            compiler_params=pltpu.CompilerParams(vmem_limit_bytes=100 * 1024 * 1024),
            name="interleaved_attention",
        )(xT, A_wq, A_wk.T, A_wv.T, A_wo, B_wqkv, B_wo)
        return jnp.transpose(out)[None]
    return jax.jit(fn)


_KERNEL = build()


@jax.jit
def pallas_interleave_layers__grouped_kv_mqa__sliding_block__prompt_kernel(
    A_x: jax.Array,
    A_wq: jax.Array,
    A_wk: jax.Array,
    A_wv: jax.Array,
    A_wo: jax.Array,
    B_x: jax.Array,
    B_wqkv: jax.Array,
    B_wo: jax.Array,
):
    return _KERNEL(A_x, A_wq, A_wk, A_wv, A_wo, B_x, B_wqkv, B_wo)
```

```python
import math

import jax
import jax.numpy as jnp
from jax import lax
import jax.experimental.pallas as pl
import jax.experimental.pallas.tpu as pltpu

S = 2048
D = 448
H = 16
DH = 28
WIN = 256
HP = 32
G = 4
GR = G * DH
NB = 4
TB = S // NB
SL = 16
QSCALE = DH ** -0.5 * math.log2(math.e)
EPS = 1e-5
F32, BF16, I32 = jnp.float32, jnp.bfloat16, jnp.int32

A_CHUNK = 128
A_LAG = 2
A_LOOPS = (((6, 2), (12, 4)), ((12, 5),))
B_LAG = 3


def _dot(a, b):
    return jnp.dot(a, b, preferred_element_type=F32)


def _words(x):
    return pltpu.bitcast(x, I32)


def _pack(x):
    return _words(x.astype(BF16))


def _bf16(x):
    return pltpu.bitcast(x, BF16)


def _recip(x):
    r = pl.reciprocal(x, approx=True)
    return r + r * (1.0 - x * r)


def _emit(main, side=()):
    done = 0
    for n, f in enumerate(main):
        f()
        while done < (n + 1) * len(side) // len(main):
            side[done]()
            done += 1


def _kernel(x_hbm, wq_hbm, wk_hbm, wv_hbm, woa_hbm, wqkv_hbm, wob_hbm, out_hbm,
            xio, wq_in, wk_in, wv_in, woa_in, wqkv_in, wob_in, sems,
            wa, woa, wb, wob, xs, xn, qs, ks, vs, att, kp, sa, sb0, sb1, sb2, zero_ref):
    @pl.loop(0, 2)
    def _(i):
        zero_ref[0] = 1 - i

    free_sems = iter(range(sems.shape[0]))

    def copy(src, dst):
        return pltpu.make_async_copy(src, dst, sems.at[next(free_sems)])

    cp_x0 = {r: copy(x_hbm.at[pl.ds(r, D // 2), pl.ds(0, TB)], xio.at[0, pl.ds(r, D // 2)]) for r in (0, D // 2)}
    cp_x = {b: copy(x_hbm.at[:, pl.ds(b * TB, TB)], xio.at[b]) for b in range(1, NB)}
    cp_first = [copy(wk_hbm, wk_in), copy(wv_hbm, wv_in),
                copy(wq_hbm.at[:, pl.ds(0, 128)], wq_in.at[:, pl.ds(0, 128)])]
    cp_wq = copy(wq_hbm.at[:, pl.ds(128, D - 128)], wq_in.at[:, pl.ds(128, D - 128)])
    cp_rest = [copy(woa_hbm, woa_in), copy(wqkv_hbm, wqkv_in), copy(wob_hbm, wob_in)]
    out_sem = sems.at[next(free_sems)]
    for cp in [*cp_x0.values(), *cp_first, cp_wq, *cp_x.values(), *cp_rest]:
        cp.start()

    def transpose_pieces(dst, src):
        def piece(c0):
            def run():
                c1 = min(c0 + 128, src.shape[1])
                dst[c0 // 2:c1 // 2, :] = _words(src[:, c0:c1].astype(BF16).T)
            return run
        return [piece(c0) for c0 in range(0, src.shape[1], 128)]

    def out_weight_pieces(dst, src):
        def piece(g):
            def run():
                w = _words(src[g * GR:(g + 1) * GR, :].astype(BF16))
                parts = []
                for j in range(G):
                    parts += [w[j * DH // 2:(j + 1) * DH // 2], jnp.zeros(((HP - DH) // 2, D), I32)]
                dst[:, g * 128:(g + 1) * 128] = _words(_bf16(jnp.concatenate(parts, axis=0)).T)
            return run
        return [piece(g) for g in range(G)]

    def kv_weights():
        pad = jnp.zeros((HP - DH, D), F32)
        wa[D // 2:D // 2 + HP, :] = _pack(
            jnp.concatenate([wk_in[...].astype(F32), pad, wv_in[...].astype(F32), pad], axis=0))

    sums = {}
    latest = []

    def add_sum(b, x):
        for r in range(0, x.shape[0], 8):
            sums[b] = sums[b] + x[r:r + 8] if b in sums else x[r:r + 8]

    def load_pieces(b):
        def piece(r0):
            def run():
                for r, cp in cp_x0.items():
                    if b == 0 and r0 <= r < r0 + 64:
                        cp.wait()
                for r in range(r0, r0 + 64, SL):
                    x = xio[b, r:r + SL].astype(F32)
                    xs[b, r:r + SL] = x
                    add_sum(b, x)
            return run
        return [piece(r0) for r0 in range(0, D, 64)]

    def paced(v):
        v = jnp.broadcast_to(v, (8, TB))
        if not latest:
            return v
        return pltpu.bitcast(pltpu.bitcast(v, I32) | (pltpu.bitcast(latest[0], I32) & zero_ref[0]), F32)

    def layernorm_pieces(b):
        st = {}

        def var_piece(r0):
            def run():
                if r0 == 0:
                    st["mean"] = jnp.sum(sums.pop(b), axis=0, keepdims=True) * (1.0 / D)
                mean = paced(st["mean"])
                for r in range(r0, r0 + SL, 8):
                    xc = xs[b, r:r + 8] - mean
                    st["var"] = xc * xc if r == 0 else st["var"] + xc * xc
            return run

        def norm_piece(r0):
            def run():
                if r0 == 0:
                    st["rstd"] = lax.rsqrt(jnp.sum(st["var"], axis=0, keepdims=True) * (1.0 / D) + EPS)
                mean = jnp.concatenate([paced(st["mean"])] * (SL // 8), axis=0)
                xn[b, r0 // 2:(r0 + SL) // 2] = _pack((xs[b, r0:r0 + SL] - mean) * st["rstd"])
            return run

        return [var_piece(r0) for r0 in range(0, D, SL)] + [norm_piece(r0) for r0 in range(0, D, SL)]

    def out_proj_pieces(b, w, sizes, last=False):
        def piece(r0, n):
            def run():
                y = _dot(_bf16(w[r0 // 2:(r0 + n) // 2]), _bf16(att[b]))
                for r in range(r0, r0 + n, SL):
                    x = xs[b, r:r + SL] + y[r - r0:r - r0 + SL]
                    if last:
                        xio[b, r:r + SL] = x.astype(xio.dtype)
                    else:
                        xs[b, r:r + SL] = x
                        add_sum(b, x)
                        latest[:] = [x[8:]]
                if last:
                    pltpu.make_async_copy(
                        xio.at[b, pl.ds(r0, n)], out_hbm.at[pl.ds(r0, n), pl.ds(b * TB, TB)], out_sem).start()
            return run
        return [piece(sum(sizes[:i]), n) for i, n in enumerate(sizes)]

    def q_pieces(b, w, rows):
        def piece(r0):
            def run():
                r1 = min(r0 + rows, D)
                y = _dot(_bf16(w[r0 // 2:r1 // 2]), _bf16(xn[b]))
                for r in range(r0, r1, SL):
                    qs[b, r // 2:(r + SL) // 2] = _pack(y[r - r0:r - r0 + SL] * QSCALE)
                latest[:] = [y[-8:]]
            return run
        return [piece(r0) for r0 in range(0, D, rows)]

    def proj_a_pieces(b, rows=64):
        def kv():
            y = _dot(_bf16(wa[D // 2:]), _bf16(xn[b]))
            row = lax.broadcasted_iota(I32, (HP, TB), 0)
            vs[0:HP // 2, b * TB:(b + 1) * TB] = _pack(jnp.where(row == DH, 1.0, y[HP:]))
            kp[b] = _pack(y[:HP])
            latest[:] = [y[-8:]]
        return [kv] + q_pieces(b, wa, rows)

    def shared_key_piece(b, j):
        def run():
            k = jnp.concatenate([kp[b], jnp.zeros(((128 - HP) // 2, TB), I32)], axis=0)
            if j:
                k = pltpu.roll(k, DH // 2 * j, 0)
            ks[j, b * TB // 2:(b + 1) * TB // 2, :] = _words(_bf16(k).T)
        return run

    def proj_b_pieces(b):
        def k_piece(g0):
            def run():
                y = _dot(_bf16(wb[(D + g0 * GR) // 2:(D + (g0 + 2) * GR) // 2]), _bf16(xn[b]))
                for n in range(2):
                    k = jnp.concatenate([y[n * GR:(n + 1) * GR], jnp.zeros((128 - GR, TB), F32)], axis=0)
                    ks[g0 + n, b * TB // 2:(b + 1) * TB // 2, :] = _words(k.astype(BF16).T)
                latest[:] = [y[-8:]]
            return run

        def v_piece(g0):
            def run():
                y = _dot(_bf16(wb[(2 * D + g0 * GR) // 2:(2 * D + (g0 + 2) * GR) // 2]), _bf16(xn[b]))
                pad = jnp.where(lax.broadcasted_iota(I32, (HP - DH, TB), 0) == 0, 1.0, 0.0).astype(F32)
                parts = []
                for h in range(2 * G):
                    parts += [y[h * DH:(h + 1) * DH], pad]
                vs[g0 * 64:(g0 + 2) * 64, b * TB:(b + 1) * TB] = _pack(jnp.concatenate(parts, axis=0))
                latest[:] = [y[-8:]]
            return run

        return q_pieces(b, wb, GR) + [k_piece(0), k_piece(2), v_piece(0), v_piece(2)]

    def attention_a(loops, weight_pieces, tail):
        nstep, nch = H * NB, S // A_CHUNK

        def aligned(r, n):
            return r if isinstance(r, int) else pl.multiple_of(r, n)

        def pv(slot, c, m, acc):
            p = jnp.exp2(sa[slot, c * A_CHUNK:(c + 1) * A_CHUNK, :] - m).astype(BF16)
            o = _dot(_bf16(vs[0:HP // 2, c * A_CHUNK:(c + 1) * A_CHUNK]), p)
            return o if acc is None else acc + o

        def step(i, slot, carry, side=()):
            m2, m1, acc = carry
            static = isinstance(i, int)
            do_qk = not static or i < nstep
            do_pv1 = not static or 1 <= i <= nstep
            do_pv2 = not static or i >= 2
            st = dict(acc=acc)
            if do_qk:
                q = qs[i >> 4, pl.ds(aligned((i >> 2 & 3) * (GR // 2), 8), GR // 2), :]
                q = _bf16(jnp.concatenate([q, jnp.zeros(((128 - GR) // 2, TB), I32)], axis=0))

            def chunk(c):
                def run():
                    if do_qk:
                        s = _dot(_bf16(ks[i & 3, c * A_CHUNK // 2:(c + 1) * A_CHUNK // 2, :]), q)
                    if c >= A_LAG:
                        if do_pv1:
                            st["acc"] = pv(1 - slot, c - A_LAG, m1, None if c == A_LAG else st["acc"])
                    elif do_pv2:
                        st["acc"] = pv(slot, nch - A_LAG + c, m2, st["acc"])
                        if c == A_LAG - 1:
                            o = st["acc"] * _recip(st["acc"][DH:DH + 1, :])
                            r0 = aligned(((i - 2) & 15) * (HP // 2), HP // 2)
                            att[(i - 2) >> 4, pl.ds(r0, HP // 2), :] = _pack(o)
                    if do_qk:
                        sa[slot, c * A_CHUNK:(c + 1) * A_CHUNK, :] = s
                        m = jnp.max(s.reshape(A_CHUNK // 8, 8, TB), axis=0)
                        st["max"] = m if c == 0 else jnp.maximum(st["max"], m)
                return run

            _emit([chunk(c) for c in range(nch if do_qk or do_pv1 else A_LAG)], side)
            return m1, jnp.max(st["max"], axis=0, keepdims=True) if do_qk else None, st["acc"]

        between = 2 if weight_pieces else 0
        first = nstep - between - sum(unroll * trips for unroll, trips in loops)
        _emit([shared_key_piece(b, 0) for b in range(NB)])
        carry = (None, None, None)
        for i in range(first):
            keys = [shared_key_piece(b, j) for j in range(1, G) if min(j, first) - 1 == i for b in range(NB)]
            carry = step(i, i % 2, carry, keys)
        latest.clear()
        for unroll, trips in loops:
            def body(it, carry, first=first, unroll=unroll):
                for u in range(unroll):
                    carry = step(first + it * unroll + u, u % 2, carry)
                return carry

            carry = lax.fori_loop(0, trips, body, carry)
            first += unroll * trips
            if between:
                for cp in cp_rest:
                    cp.wait()
                n = len(weight_pieces)
                for u in range(between):
                    carry = step(first + u, u % 2, carry, weight_pieces[u * n // between:(u + 1) * n // between])
                first, between = first + between, 0
        carry = step(nstep, 0, carry, tail[:-2])
        step(nstep + 1, 1, carry, tail[-2:])

    def attention_b(tail):
        bl = 128 // G
        tpb = TB // 128
        lane = lax.broadcasted_iota(I32, (8, 128), 1)
        sub = lax.broadcasted_iota(I32, (8, 128), 0)
        zero = jnp.zeros((8, 128), I32)
        in_first_band = (lax.broadcasted_iota(I32, (bl, 128), 0)
                         > (lax.broadcasted_iota(I32, (bl, 128), 1) & (bl - 1)))
        in_block = [(lane >= bl * n) & (lane < bl * (n + 1)) for n in range(G)]
        chunks = [[(bl, 3 * bl)], [(0, bl), (WIN, bl), (4 * bl, bl)], [(5 * bl, 3 * bl)]]

        def queries(g, t):
            q = qs[t // tpb, g * GR // 2:(g + 1) * GR // 2, (t % tpb) * 128:(t % tpb + 1) * 128]
            cols = [[] for _ in range(G)]
            for r in range(0, GR // 2, 8):
                x = q[r:r + 8]
                j0, j1 = r // (DH // 2), (r + 7) // (DH // 2)
                x0 = pltpu.roll(x, bl * j0, 1) if j0 else x
                if j0 != j1:
                    low = sub < j1 * (DH // 2) - r
                    x0 = lax.select(low, x0, pltpu.roll(x, bl * j1, 1))
                for u in range(G):
                    keep = in_block[(j0 + u) % G]
                    if j0 != j1:
                        keep = (keep & low) | (in_block[(j1 + u) % G] & ~low)
                    cols[u].append(lax.select(keep, x0, zero))
            return [_bf16(jnp.concatenate(col + [zero], axis=0)) for col in cols]

        def scores(buf, g, t, c, st):
            def put(u, r, s):
                buf[0, u, r:r + s.shape[0], :] = s
                for n in range(0, s.shape[0], 8):
                    st["max"][u] = s[n:n + 8] if st["max"][u] is None else lax.max(st["max"][u], s[n:n + 8])

            if t >= 2:
                for u in range(G):
                    k0 = 128 * t + bl * u - WIN
                    k = [ks[g, (k0 + r) // 2:(k0 + r + n) // 2, :] for r, n in chunks[c]]
                    s = _dot(_bf16(jnp.concatenate(k, axis=0)), st["q"][u])
                    if len(k) > 1:
                        put(u, 0, jnp.where(in_first_band, s[:bl], s[bl:2 * bl]))
                    r, n = chunks[c][-1]
                    put(u, r, s[-n:])
            elif c <= t:
                s = _dot(_bf16(ks[g, 64 * c:64 * (c + 1), :]), jnp.concatenate(st["q"], axis=1))
                for u in range(G):
                    su = s[:, 128 * u:128 * (u + 1)]
                    n = 128 if c < t else bl * u
                    if n:
                        put(u, WIN - 128 * (t - c) - bl * u, su[:n])
                    if c == t:
                        put(u, 0, jnp.where(in_first_band, -jnp.inf, su[n:n + bl]))
            if c == 2:
                st["max"] = [jnp.max(m, axis=0, keepdims=True) for m in st["max"]]

        def pv(buf, g, t, n, st):
            c = (1, 0, 2)[n]
            kt = t - 2 + c
            if kt >= 0:
                z = zero_ref[0]
                col = lax.broadcasted_iota(I32, (128, 128), 1) + z
                odd, high = col & bl != 0, col & (2 * bl) != 0
                x = []
                for u in range(G):
                    def weights(r0, r1):
                        return jnp.exp2(buf[z, u, r0:r1, :] - st["max"][u])

                    r0, r1 = 128 * c - bl * u, 128 * (c + 1) - bl * u
                    parts = [weights(max(r0, bl), min(r1, WIN))] if max(r0, bl) < min(r1, WIN) else []
                    if r0 <= 0:
                        band = weights(0, bl)
                        parts = [jnp.where(in_first_band, band, 0.0)] + parts
                        st["last"][u] = jnp.where(in_first_band, 0.0, band)
                    if r0 < 0:
                        parts = [jnp.zeros((-r0, 128), F32)] + parts
                    if r1 > WIN:
                        parts.append(st["last"][u] if t >= 2 else weights(0, bl))
                    if r1 > WIN + bl:
                        parts.append(jnp.zeros((r1 - WIN - bl, 128), F32))
                    x.append(jnp.concatenate(parts, axis=0))
                a = [jnp.where(odd, x[(v + 1) % G], x[v]) for v in range(G)]
                p = [jnp.where(high, a[(2 - j) % G], a[-j % G]) for j in range(G)]
                acc = []
                for j in range(G):
                    r0 = (g * G + j) * HP // 2
                    o = _dot(_bf16(vs[r0:r0 + HP // 2, kt * 128:(kt + 1) * 128]), p[j].astype(BF16))
                    acc.append(o if st["acc"] is None else o + st["acc"][j])
                st["acc"] = acc
            if n == 2:
                o = jnp.concatenate(st["acc"], axis=1)
                o = _pack(o * _recip(o[DH:DH + 1, :]))
                for j in range(G):
                    oj = o[:, j * 128:(j + 1) * 128]
                    r0 = (g * G + j) * HP // 2
                    att[t // tpb, r0:r0 + HP // 2, (t % tpb) * 128:(t % tpb + 1) * 128] = (
                        pltpu.roll(oj, 128 - bl * j, 1) if j else oj)

        tiles = [(g, t) for b in range(NB) for g in range(G) for t in range(tpb * b, tpb * (b + 1))]
        bufs, state = (sb0, sb1, sb2), {}

        def slot(k):
            def run():
                i, c = divmod(k, 3)
                if i < len(tiles):
                    if c == 0:
                        state[i] = dict(max=[None] * G, acc=None, last={}, q=queries(*tiles[i]))
                    scores(bufs[i % 3], *tiles[i], c, state[i])
                i, c = divmod(k - 3 - B_LAG, 3)
                if i >= 0:
                    pv(bufs[i % 3], *tiles[i], c, state[i])
            return run

        _emit([slot(k) for k in range(3 * len(tiles))])
        _emit([slot(k) for k in range(3 * len(tiles), 3 * len(tiles) + 3 + B_LAG)], tail)

    def transition(w, proj, extra=()):
        _emit(out_proj_pieces(2, w, (GR,) * G) + out_proj_pieces(3, w, (GR,) * G), layernorm_pieces(0))
        for b in range(NB):
            _emit(proj(b), layernorm_pieces(b + 1) if b + 1 < NB else extra)

    _emit(load_pieces(0) + layernorm_pieces(0))
    for cp in cp_first:
        cp.wait()
    kv_weights()
    proj, wq = proj_a_pieces(0, 128), transpose_pieces(wa, wq_in)
    _emit(wq[:1] + proj[:2])
    cp_wq.wait()
    _emit(wq[1:] + proj[2:3])
    cp_x[1].wait()
    _emit(proj[3:], load_pieces(1) + layernorm_pieces(1))
    for b in range(1, NB - 1):
        cp_x[b + 1].wait()
        _emit(proj_a_pieces(b), load_pieces(b + 1) + layernorm_pieces(b + 1))
    _emit(proj_a_pieces(NB - 1))

    for last in (False, True):
        attention_a(A_LOOPS[last],
                    [] if last else out_weight_pieces(woa, woa_in) + transpose_pieces(wb, wqkv_in),
                    out_proj_pieces(0, woa, (64,) * 7) + out_proj_pieces(1, woa, (64,) * 7))
        transition(woa, proj_b_pieces, [] if last else out_weight_pieces(wob, wob_in))
        attention_b(out_proj_pieces(0, wob, (GR,) * G, last) + out_proj_pieces(1, wob, (GR,) * G, last))
        if not last:
            transition(wob, proj_a_pieces)
    _emit(out_proj_pieces(2, wob, (GR,) * G, True) + out_proj_pieces(3, wob, (160, 128, 96, 32, 32), True))
    pltpu.make_async_copy(out_hbm, out_hbm, out_sem).wait()


def _forward(A_x, A_wq, A_wk, A_wv, A_wo, B_wqkv, B_wo, **call_args):
    out = pl.pallas_call(
        _kernel,
        out_shape=jax.ShapeDtypeStruct((D, S), A_x.dtype),
        in_specs=[pl.BlockSpec(memory_space=pl.ANY)] * 7,
        out_specs=pl.BlockSpec(memory_space=pl.ANY),
        scratch_shapes=[
            pltpu.VMEM((NB, D, TB), A_x.dtype),
            pltpu.VMEM((D, D), A_wq.dtype),
            pltpu.VMEM((DH, D), A_wk.dtype),
            pltpu.VMEM((DH, D), A_wv.dtype),
            pltpu.VMEM((D, D), A_wo.dtype),
            pltpu.VMEM((D, 3 * D), B_wqkv.dtype),
            pltpu.VMEM((D, D), B_wo.dtype),
            pltpu.SemaphoreType.DMA((13,)),
            pltpu.VMEM((D // 2 + HP, D), I32),
            pltpu.VMEM((D // 2, H * HP), I32),
            pltpu.VMEM((3 * D // 2, D), I32),
            pltpu.VMEM((D // 2, H * HP), I32),
            pltpu.VMEM((NB, D, TB), F32),
            pltpu.VMEM((NB, D // 2, TB), I32),
            pltpu.VMEM((NB, D // 2, TB), I32),
            pltpu.VMEM((G, S // 2, 128), I32),
            pltpu.VMEM((H * HP // 2, S), I32),
            pltpu.VMEM((NB, H * HP // 2, TB), I32),
            pltpu.VMEM((NB, HP // 2, TB), I32),
            pltpu.VMEM((2, S, TB), F32),
            pltpu.VMEM((1, G, WIN, 128), F32),
            pltpu.VMEM((1, G, WIN, 128), F32),
            pltpu.VMEM((1, G, WIN, 128), F32),
            pltpu.SMEM((1,), I32),
        ],
        compiler_params=pltpu.CompilerParams(vmem_limit_bytes=100 * 1024 * 1024),
        name="interleaved_attention",
        **call_args,
    )(A_x[0].T, A_wq, A_wk.T, A_wv.T, A_wo, B_wqkv, B_wo)
    return out.T[None]


@jax.jit
def pallas_interleave_layers__grouped_kv_mqa__sliding_block__prompt_kernel(
    A_x: jax.Array,
    A_wq: jax.Array,
    A_wk: jax.Array,
    A_wv: jax.Array,
    A_wo: jax.Array,
    B_x: jax.Array,
    B_wqkv: jax.Array,
    B_wo: jax.Array,
):
    del B_x
    return _forward(A_x, A_wq, A_wk, A_wv, A_wo, B_wqkv, B_wo)
```

```python
import math

import jax
import jax.numpy as jnp
from jax import lax
import jax.experimental.pallas as pl
import jax.experimental.pallas.tpu as pltpu

S = 2048
D = 448
H = 16
DH = 28
WIN = 256
HP = 32
G = 4
GR = G * DH
NB = 4
TB = S // NB
SL = 16
QSCALE = DH ** -0.5 * math.log2(math.e)
EPS = 1e-5
F32, BF16, I32 = jnp.float32, jnp.bfloat16, jnp.int32

A_CHUNK = 128
A_LAG = 1
A_LOOPS = (((6, 2), (12, 4)), ((12, 5),))
B_LAG = 3


def _dot(a, b):
    return jnp.dot(a, b, preferred_element_type=F32)


def _words(x):
    return pltpu.bitcast(x, I32)


def _pack(x):
    return _words(x.astype(BF16))


def _bf16(x):
    return pltpu.bitcast(x, BF16)


def _recip(x):
    r = pl.reciprocal(x, approx=True)
    return r + r * (1.0 - x * r)


def _emit(main, side=()):
    done = 0
    for n, f in enumerate(main):
        f()
        while done < (n + 1) * len(side) // len(main):
            side[done]()
            done += 1


def _kernel(x_hbm, wq_hbm, wk_hbm, wv_hbm, woa_hbm, wqkv_hbm, wob_hbm, out_hbm,
            xio, wq_in, wk_in, wv_in, woa_in, wqkv_in, wob_in, sems,
            wa, woa, wb, wob, xs, xn, qs, ks, vs, att, kp, sa, sb0, sb1, sb2, zero_ref):
    @pl.loop(0, 2)
    def _(i):
        zero_ref[0] = 1 - i

    free_sems = iter(range(sems.shape[0]))

    def copy(src, dst):
        return pltpu.make_async_copy(src, dst, sems.at[next(free_sems)])

    cp_x0 = {r: copy(x_hbm.at[pl.ds(r, D // 2), pl.ds(0, TB)], xio.at[0, pl.ds(r, D // 2)]) for r in (0, D // 2)}
    cp_x = {b: copy(x_hbm.at[:, pl.ds(b * TB, TB)], xio.at[b]) for b in range(1, NB)}
    cp_first = [copy(wk_hbm, wk_in), copy(wv_hbm, wv_in),
                copy(wq_hbm.at[:, pl.ds(0, 128)], wq_in.at[:, pl.ds(0, 128)])]
    cp_wq = copy(wq_hbm.at[:, pl.ds(128, D - 128)], wq_in.at[:, pl.ds(128, D - 128)])
    cp_rest = [copy(woa_hbm, woa_in), copy(wqkv_hbm, wqkv_in), copy(wob_hbm, wob_in)]
    out_sem = sems.at[next(free_sems)]
    for cp in [*cp_x0.values(), *cp_first, cp_wq, *cp_x.values(), *cp_rest]:
        cp.start()

    def transpose_pieces(dst, src):
        def piece(c0):
            def run():
                c1 = min(c0 + 128, src.shape[1])
                dst[c0 // 2:c1 // 2, :] = _words(src[:, c0:c1].astype(BF16).T)
            return run
        return [piece(c0) for c0 in range(0, src.shape[1], 128)]

    def out_weight_pieces(dst, src):
        def piece(g):
            def run():
                w = _words(src[g * GR:(g + 1) * GR, :].astype(BF16))
                parts = []
                for j in range(G):
                    parts += [w[j * DH // 2:(j + 1) * DH // 2], jnp.zeros(((HP - DH) // 2, D), I32)]
                dst[:, g * 128:(g + 1) * 128] = _words(_bf16(jnp.concatenate(parts, axis=0)).T)
            return run
        return [piece(g) for g in range(G)]

    def kv_weights():
        pad = jnp.zeros((HP - DH, D), F32)
        wa[D // 2:D // 2 + HP, :] = _pack(
            jnp.concatenate([wk_in[...].astype(F32), pad, wv_in[...].astype(F32), pad], axis=0))

    sums = {}
    latest = []

    def add_sum(b, x):
        for r in range(0, x.shape[0], 8):
            sums[b] = sums[b] + x[r:r + 8] if b in sums else x[r:r + 8]

    def load_pieces(b):
        def piece(r0):
            def run():
                for r, cp in cp_x0.items():
                    if b == 0 and r0 <= r < r0 + 64:
                        cp.wait()
                for r in range(r0, r0 + 64, SL):
                    x = xio[b, r:r + SL].astype(F32)
                    xs[b, r:r + SL] = x
                    add_sum(b, x)
            return run
        return [piece(r0) for r0 in range(0, D, 64)]

    def paced(v):
        v = jnp.broadcast_to(v, (8, TB))
        if not latest:
            return v
        return pltpu.bitcast(pltpu.bitcast(v, I32) | (pltpu.bitcast(latest[0], I32) & zero_ref[0]), F32)

    def layernorm_pieces(b):
        st = {}

        def var_piece(r0):
            def run():
                if r0 == 0:
                    st["mean"] = jnp.sum(sums.pop(b), axis=0, keepdims=True) * (1.0 / D)
                mean = paced(st["mean"])
                for r in range(r0, r0 + SL, 8):
                    xc = xs[b, r:r + 8] - mean
                    st["var"] = xc * xc if r == 0 else st["var"] + xc * xc
            return run

        def norm_piece(r0):
            def run():
                if r0 == 0:
                    st["rstd"] = lax.rsqrt(jnp.sum(st["var"], axis=0, keepdims=True) * (1.0 / D) + EPS)
                mean = jnp.concatenate([paced(st["mean"])] * (SL // 8), axis=0)
                xn[b, r0 // 2:(r0 + SL) // 2] = _pack((xs[b, r0:r0 + SL] - mean) * st["rstd"])
            return run

        return [var_piece(r0) for r0 in range(0, D, SL)] + [norm_piece(r0) for r0 in range(0, D, SL)]

    def out_proj_pieces(b, w, last=False, sizes=(GR,) * G):
        def piece(r0, n):
            def run():
                y = _dot(_bf16(w[r0 // 2:(r0 + n) // 2]), _bf16(att[b]))
                for r in range(r0, r0 + n, SL):
                    x = xs[b, r:r + SL] + y[r - r0:r - r0 + SL]
                    if last:
                        xio[b, r:r + SL] = x.astype(xio.dtype)
                    else:
                        xs[b, r:r + SL] = x
                        add_sum(b, x)
                        latest[:] = [x[8:]]
                if last:
                    pltpu.make_async_copy(
                        xio.at[b, pl.ds(r0, n)], out_hbm.at[pl.ds(r0, n), pl.ds(b * TB, TB)], out_sem).start()
            return run
        return [piece(sum(sizes[:i]), n) for i, n in enumerate(sizes)]

    def q_pieces(b, w, rows):
        def piece(r0):
            def run():
                r1 = min(r0 + rows, D)
                y = _dot(_bf16(w[r0 // 2:r1 // 2]), _bf16(xn[b]))
                for r in range(r0, r1, SL):
                    qs[b, r // 2:(r + SL) // 2] = _pack(y[r - r0:r - r0 + SL] * QSCALE)
                latest[:] = [y[-8:]]
            return run
        return [piece(r0) for r0 in range(0, D, rows)]

    def proj_a_pieces(b, rows=64):
        def kv():
            y = _dot(_bf16(wa[D // 2:]), _bf16(xn[b]))
            row = lax.broadcasted_iota(I32, (HP, TB), 0)
            vs[0:HP // 2, b * TB:(b + 1) * TB] = _pack(jnp.where(row == DH, 1.0, y[HP:]))
            kp[b] = _pack(y[:HP])
            latest[:] = [y[-8:]]
        return [kv] + q_pieces(b, wa, rows)

    def shared_key_piece(b, j):
        def run():
            k = jnp.concatenate([kp[b], jnp.zeros(((128 - HP) // 2, TB), I32)], axis=0)
            if j:
                k = pltpu.roll(k, DH // 2 * j, 0)
            ks[j, b * TB // 2:(b + 1) * TB // 2, :] = _words(_bf16(k).T)
        return run

    def proj_b_pieces(b):
        def k_piece(g0):
            def run():
                y = _dot(_bf16(wb[(D + g0 * GR) // 2:(D + (g0 + 2) * GR) // 2]), _bf16(xn[b]))
                for n in range(2):
                    k = jnp.concatenate([y[n * GR:(n + 1) * GR], jnp.zeros((128 - GR, TB), F32)], axis=0)
                    ks[g0 + n, b * TB // 2:(b + 1) * TB // 2, :] = _words(k.astype(BF16).T)
                latest[:] = [y[-8:]]
            return run

        def v_piece(g0):
            def run():
                y = _dot(_bf16(wb[(2 * D + g0 * GR) // 2:(2 * D + (g0 + 2) * GR) // 2]), _bf16(xn[b]))
                pad = jnp.where(lax.broadcasted_iota(I32, (HP - DH, TB), 0) == 0, 1.0, 0.0).astype(F32)
                parts = []
                for h in range(2 * G):
                    parts += [y[h * DH:(h + 1) * DH], pad]
                vs[g0 * 64:(g0 + 2) * 64, b * TB:(b + 1) * TB] = _pack(jnp.concatenate(parts, axis=0))
                latest[:] = [y[-8:]]
            return run

        return q_pieces(b, wb, GR) + [k_piece(0), k_piece(2), v_piece(0), v_piece(2)]

    def attention_a(loops, weight_pieces, tail):
        nstep, nch = H * NB, S // A_CHUNK

        def aligned(r, n):
            return r if isinstance(r, int) else pl.multiple_of(r, n)

        def pv(slot, c, m, acc):
            p = jnp.exp2(sa[slot, c * A_CHUNK:(c + 1) * A_CHUNK, :] - m).astype(BF16)
            o = _dot(_bf16(vs[0:HP // 2, c * A_CHUNK:(c + 1) * A_CHUNK]), p)
            return o if acc is None else acc + o

        def step(i, slot, carry, side=()):
            m2, m1, acc = carry
            if m1 is not None:
                m1 = jnp.max(m1, axis=0, keepdims=True)
            static = isinstance(i, int)
            do_qk = not static or i < nstep
            do_pv1 = not static or 1 <= i <= nstep
            do_pv2 = not static or i >= 2
            st = dict(acc=acc)
            if do_qk:
                q = qs[i >> 4, pl.ds(aligned((i >> 2 & 3) * (GR // 2), 8), GR // 2), :]
                q = _bf16(jnp.concatenate([q, jnp.zeros(((128 - GR) // 2, TB), I32)], axis=0))

            def chunk(c):
                def run():
                    if do_qk:
                        s = _dot(_bf16(ks[i & 3, c * A_CHUNK // 2:(c + 1) * A_CHUNK // 2, :]), q)
                    if c >= A_LAG:
                        if do_pv1:
                            st["acc"] = pv(1 - slot, c - A_LAG, m1, None if c == A_LAG else st["acc"])
                    elif do_pv2:
                        st["acc"] = pv(slot, nch - A_LAG + c, m2, st["acc"])
                        if c == A_LAG - 1:
                            o = st["acc"] * _recip(st["acc"][DH:DH + 1, :])
                            r0 = aligned(((i - 2) & 15) * (HP // 2), HP // 2)
                            att[(i - 2) >> 4, pl.ds(r0, HP // 2), :] = _pack(o)
                    if do_qk:
                        sa[slot, c * A_CHUNK:(c + 1) * A_CHUNK, :] = s
                        for r in range(0, A_CHUNK, 8):
                            st["max"] = lax.max(st["max"], s[r:r + 8]) if "max" in st else s[r:r + 8]
                return run

            _emit([chunk(c) for c in range(nch if do_qk or do_pv1 else A_LAG)], side)
            return m1, st.get("max"), st["acc"]

        between = 2 if weight_pieces else 0
        first = nstep - between - sum(unroll * trips for unroll, trips in loops)
        _emit([shared_key_piece(b, 0) for b in range(NB)])
        carry = (None, None, None)
        for i in range(first):
            keys = [shared_key_piece(b, j) for j in range(1, G) if min(j, first) - 1 == i for b in range(NB)]
            carry = step(i, i % 2, carry, keys)
        latest.clear()
        for unroll, trips in loops:
            def body(it, carry, first=first, unroll=unroll):
                for u in range(unroll):
                    carry = step(first + it * unroll + u, u % 2, carry)
                return carry

            carry = lax.fori_loop(0, trips, body, carry)
            first += unroll * trips
            if between:
                for cp in cp_rest:
                    cp.wait()
                n = len(weight_pieces)
                for u in range(between):
                    carry = step(first + u, u % 2, carry, weight_pieces[u * n // between:(u + 1) * n // between])
                first, between = first + between, 0
        _emit(tail[:1])
        carry = step(nstep, 0, carry, tail[1:])
        step(nstep + 1, 1, carry)

    def attention_b(tail):
        bl = 128 // G
        tpb = TB // 128
        lane = lax.broadcasted_iota(I32, (8, 128), 1)
        sub = lax.broadcasted_iota(I32, (8, 128), 0)
        zero = jnp.zeros((8, 128), I32)
        in_first_band = (lax.broadcasted_iota(I32, (bl, 128), 0)
                         > (lax.broadcasted_iota(I32, (bl, 128), 1) & (bl - 1)))
        in_block = [(lane >= bl * n) & (lane < bl * (n + 1)) for n in range(G)]
        chunks = [[(bl, 3 * bl)], [(0, bl), (WIN, bl), (4 * bl, bl)], [(5 * bl, 3 * bl)]]

        def queries(g, t):
            q = qs[t // tpb, g * GR // 2:(g + 1) * GR // 2, (t % tpb) * 128:(t % tpb + 1) * 128]
            cols = [[] for _ in range(G)]
            for r in range(0, GR // 2, 8):
                x = q[r:r + 8]
                j0, j1 = r // (DH // 2), (r + 7) // (DH // 2)
                x0 = pltpu.roll(x, bl * j0, 1) if j0 else x
                if j0 != j1:
                    low = sub < j1 * (DH // 2) - r
                    x0 = lax.select(low, x0, pltpu.roll(x, bl * j1, 1))
                for u in range(G):
                    keep = in_block[(j0 + u) % G]
                    if j0 != j1:
                        keep = (keep & low) | (in_block[(j1 + u) % G] & ~low)
                    cols[u].append(lax.select(keep, x0, zero))
            return [_bf16(jnp.concatenate(col + [zero], axis=0)) for col in cols]

        def scores(buf, g, t, c, st):
            def put(u, r, s):
                buf[0, u, r:r + s.shape[0], :] = s
                for n in range(0, s.shape[0], 8):
                    st["max"][u] = s[n:n + 8] if st["max"][u] is None else lax.max(st["max"][u], s[n:n + 8])

            if t >= 2:
                for u in range(G):
                    k0 = 128 * t + bl * u - WIN
                    k = [ks[g, (k0 + r) // 2:(k0 + r + n) // 2, :] for r, n in chunks[c]]
                    s = _dot(_bf16(jnp.concatenate(k, axis=0)), st["q"][u])
                    if len(k) > 1:
                        put(u, 0, jnp.where(in_first_band, s[:bl], s[bl:2 * bl]))
                    r, n = chunks[c][-1]
                    put(u, r, s[-n:])
            elif c <= t:
                s = _dot(_bf16(ks[g, 64 * c:64 * (c + 1), :]), jnp.concatenate(st["q"], axis=1))
                for u in range(G):
                    su = s[:, 128 * u:128 * (u + 1)]
                    n = 128 if c < t else bl * u
                    if n:
                        put(u, WIN - 128 * (t - c) - bl * u, su[:n])
                    if c == t:
                        put(u, 0, jnp.where(in_first_band, -jnp.inf, su[n:n + bl]))
            if c == 2:
                st["max"] = [jnp.max(m, axis=0, keepdims=True) for m in st["max"]]

        def pv(buf, g, t, n, st):
            c = (1, 0, 2)[n]
            kt = t - 2 + c
            if kt >= 0:
                z = zero_ref[0]
                col = lax.broadcasted_iota(I32, (128, 128), 1) + z
                odd, high = col & bl != 0, col & (2 * bl) != 0
                x = []
                for u in range(G):
                    def weights(r0, r1):
                        return jnp.exp2(buf[z, u, r0:r1, :] - st["max"][u])

                    r0, r1 = 128 * c - bl * u, 128 * (c + 1) - bl * u
                    parts = [weights(max(r0, bl), min(r1, WIN))] if max(r0, bl) < min(r1, WIN) else []
                    if r0 <= 0:
                        band = weights(0, bl)
                        parts = [jnp.where(in_first_band, band, 0.0)] + parts
                        st["last"][u] = jnp.where(in_first_band, 0.0, band)
                    if r0 < 0:
                        parts = [jnp.zeros((-r0, 128), F32)] + parts
                    if r1 > WIN:
                        parts.append(st["last"][u] if t >= 2 else weights(0, bl))
                    if r1 > WIN + bl:
                        parts.append(jnp.zeros((r1 - WIN - bl, 128), F32))
                    x.append(jnp.concatenate(parts, axis=0))
                a = [jnp.where(odd, x[(v + 1) % G], x[v]) for v in range(G)]
                p = [jnp.where(high, a[(2 - j) % G], a[-j % G]) for j in range(G)]
                acc = []
                for j in range(G):
                    r0 = (g * G + j) * HP // 2
                    o = _dot(_bf16(vs[r0:r0 + HP // 2, kt * 128:(kt + 1) * 128]), p[j].astype(BF16))
                    acc.append(o if st["acc"] is None else o + st["acc"][j])
                st["acc"] = acc
            if n == 2:
                o = jnp.concatenate(st["acc"], axis=1)
                o = _pack(o * _recip(o[DH:DH + 1, :]))
                for j in range(G):
                    oj = o[:, j * 128:(j + 1) * 128]
                    r0 = (g * G + j) * HP // 2
                    att[t // tpb, r0:r0 + HP // 2, (t % tpb) * 128:(t % tpb + 1) * 128] = (
                        pltpu.roll(oj, 128 - bl * j, 1) if j else oj)

        tiles = [(g, t) for t in range(S // 128) for g in range(G)]
        bufs, state = (sb0, sb1, sb2), {}

        def slot(k):
            def run():
                i, c = divmod(k, 3)
                if i < len(tiles):
                    if c == 0:
                        state[i] = dict(max=[None] * G, acc=None, last={}, q=queries(*tiles[i]))
                    scores(bufs[i % 3], *tiles[i], c, state[i])
                i, c = divmod(k - 3 - B_LAG, 3)
                if i >= 0:
                    pv(bufs[i % 3], *tiles[i], c, state[i])
            return run

        _emit([slot(k) for k in range(3 * len(tiles))])
        _emit([slot(k) for k in range(3 * len(tiles), 3 * len(tiles) + 3 + B_LAG)], tail)

    def transition(w, proj, extra=()):
        _emit(out_proj_pieces(2, w) + out_proj_pieces(3, w), layernorm_pieces(0))
        for b in range(NB):
            _emit(proj(b), layernorm_pieces(b + 1) if b + 1 < NB else extra)

    _emit(load_pieces(0) + layernorm_pieces(0))
    for cp in cp_first:
        cp.wait()
    kv_weights()
    proj, wq = proj_a_pieces(0, 128), transpose_pieces(wa, wq_in)
    _emit(wq[:1] + proj[:2])
    cp_wq.wait()
    _emit(wq[1:] + proj[2:3])
    cp_x[1].wait()
    _emit(proj[3:], load_pieces(1) + layernorm_pieces(1))
    for b in range(1, NB - 1):
        cp_x[b + 1].wait()
        _emit(proj_a_pieces(b), load_pieces(b + 1) + layernorm_pieces(b + 1))
    _emit(proj_a_pieces(NB - 1))

    for last in (False, True):
        attention_a(A_LOOPS[last],
                    [] if last else out_weight_pieces(woa, woa_in) + transpose_pieces(wb, wqkv_in),
                    out_proj_pieces(0, woa) + out_proj_pieces(1, woa))
        transition(woa, proj_b_pieces, [] if last else out_weight_pieces(wob, wob_in))
        attention_b(out_proj_pieces(0, wob, last) + out_proj_pieces(1, wob, last))
        if not last:
            transition(wob, proj_a_pieces)
    _emit(out_proj_pieces(2, wob, True) + out_proj_pieces(3, wob, True, (160, 128, 96, 32, 32)))
    pltpu.make_async_copy(out_hbm, out_hbm, out_sem).wait()


def _forward(A_x, A_wq, A_wk, A_wv, A_wo, B_wqkv, B_wo, **call_args):
    out = pl.pallas_call(
        _kernel,
        out_shape=jax.ShapeDtypeStruct((D, S), A_x.dtype),
        in_specs=[pl.BlockSpec(memory_space=pl.ANY)] * 7,
        out_specs=pl.BlockSpec(memory_space=pl.ANY),
        scratch_shapes=[
            pltpu.VMEM((NB, D, TB), A_x.dtype),
            pltpu.VMEM((D, D), A_wq.dtype),
            pltpu.VMEM((DH, D), A_wk.dtype),
            pltpu.VMEM((DH, D), A_wv.dtype),
            pltpu.VMEM((D, D), A_wo.dtype),
            pltpu.VMEM((D, 3 * D), B_wqkv.dtype),
            pltpu.VMEM((D, D), B_wo.dtype),
            pltpu.SemaphoreType.DMA((13,)),
            pltpu.VMEM((D // 2 + HP, D), I32),
            pltpu.VMEM((D // 2, H * HP), I32),
            pltpu.VMEM((3 * D // 2, D), I32),
            pltpu.VMEM((D // 2, H * HP), I32),
            pltpu.VMEM((NB, D, TB), F32),
            pltpu.VMEM((NB, D // 2, TB), I32),
            pltpu.VMEM((NB, D // 2, TB), I32),
            pltpu.VMEM((G, S // 2, 128), I32),
            pltpu.VMEM((H * HP // 2, S), I32),
            pltpu.VMEM((NB, H * HP // 2, TB), I32),
            pltpu.VMEM((NB, HP // 2, TB), I32),
            pltpu.VMEM((2, S, TB), F32),
            pltpu.VMEM((1, G, WIN, 128), F32),
            pltpu.VMEM((1, G, WIN, 128), F32),
            pltpu.VMEM((1, G, WIN, 128), F32),
            pltpu.SMEM((1,), I32),
        ],
        compiler_params=pltpu.CompilerParams(vmem_limit_bytes=100 * 1024 * 1024),
        name="interleaved_attention",
        **call_args,
    )(A_x[0].T, A_wq, A_wk.T, A_wv.T, A_wo, B_wqkv, B_wo)
    return out.T[None]


@jax.jit
def pallas_interleave_layers__grouped_kv_mqa__sliding_block__prompt_kernel(
    A_x: jax.Array,
    A_wq: jax.Array,
    A_wk: jax.Array,
    A_wv: jax.Array,
    A_wo: jax.Array,
    B_x: jax.Array,
    B_wqkv: jax.Array,
    B_wo: jax.Array,
):
    del B_x
    return _forward(A_x, A_wq, A_wk, A_wv, A_wo, B_wqkv, B_wo)
```
